```python
import jax
import jax.numpy as jnp

def _softmax(x, axis=-1):
    return jax.nn.softmax(x, axis=axis)
def _gelu(x):
    return jax.nn.gelu(x, approximate=True)
def _silu(x):
    return jax.nn.silu(x)
def _sigmoid(x):
    return jax.nn.sigmoid(x)
def _layernorm(x, axis=-1, eps=1e-5):
    m = jnp.mean(x, axis=axis, keepdims=True)
    v = jnp.var(x, axis=axis, keepdims=True)
    return (x - m) / jnp.sqrt(v + eps)
def _scatter_add(tgt, idx, src, axis=0):
    return tgt.at[idx].add(src)
def _segment_sum(src, seg, n):
    return jax.ops.segment_sum(src, seg, n)
class _Rng:
    def __init__(self, key):
        self._k = key
    def _next(self):
        self._k, sub = jax.random.split(self._k)
        return sub
    def normal(self, shape):
        return jax.random.normal(self._next(), shape, dtype=jnp.bfloat16)
    def randint(self, lo, hi, shape):
        return jax.random.randint(self._next(), shape, lo, hi, dtype=jnp.int32)
    def uniform(self, shape, lo=0.0, hi=1.0):
        return jax.random.uniform(self._next(), shape, jnp.bfloat16, lo, hi)
    def permutation(self, n):
        return jax.random.permutation(self._next(), n)


kernel_name = 'recurrent_scan__compressed_kv_cla__dense_activation_gelu__decode'

def setup_inputs():
    _rng = _Rng(jax.random.key(int.from_bytes(__import__("os").urandom(4), "little")))
    _w = (lambda a: (lambda t: t.astype(jnp.bfloat16) if jnp.issubdtype(t.dtype, jnp.floating) else t)(jnp.asarray(a)))
    def _A_setup():
        B, H, Sq, Sk, D, M = 2, 32, 1, 16384, 128, 512
        Dc = 4 * D
        return {
            "x": _w((lambda *s: _rng.normal(s) * 0.05)(B, Sq, M)),
            "c_kv": _w((lambda *s: _rng.normal(s) * 0.05)(B, Sk, Dc)),
            "w_q": _w((lambda *s: _rng.normal(s) * 0.05)(M, H, D) * (M ** -0.5)),
            "w_uk": _w((lambda *s: _rng.normal(s) * 0.05)(Dc, H, D) * (Dc ** -0.5)),
            "w_uv": _w((lambda *s: _rng.normal(s) * 0.05)(Dc, H, D) * (Dc ** -0.5)),
            "w_o": _w((lambda *s: _rng.normal(s) * 0.05)(H, D, M) * ((H * D) ** -0.5)),
        }
    _A_in = _A_setup()

    def _B_setup():
        B, S, D, F = 2, 1, 512, 1792
        return {
            "x": _w((lambda *s: _rng.normal(s) * 0.05)(B, S, D)),
            "w1": _w((lambda *s: _rng.normal(s) * 0.05)(D, F) * (D ** -0.5)),
            "b1": _w((lambda *s: _rng.normal(s) * 0.05)(F) * 0.01),
            "w2": _w((lambda *s: _rng.normal(s) * 0.05)(F, D) * (F ** -0.5)),
            "b2": _w((lambda *s: _rng.normal(s) * 0.05)(D) * 0.01),
        }
    _B_in = _B_setup()

    return {
        "A_x": _A_in["x"],
        "A_c_kv": _A_in["c_kv"],
        "A_w_q": _A_in["w_q"],
        "A_w_uk": _A_in["w_uk"],
        "A_w_uv": _A_in["w_uv"],
        "A_w_o": _A_in["w_o"],
        "B_x": _B_in["x"],
        "B_w1": _B_in["w1"],
        "B_b1": _B_in["b1"],
        "B_w2": _B_in["w2"],
        "B_b2": _B_in["b2"],
    }

def reference(A_x, A_c_kv, A_w_q, A_w_uk, A_w_uv, A_w_o, B_x, B_w1, B_b1, B_w2, B_b2):
    def _A_ref(x, c_kv, w_q, w_uk, w_uv, w_o):
        B, Sq, M = x.shape[0], x.shape[1], x.shape[2]
        Sk = c_kv.shape[1]
        H, D = w_q.shape[1], w_q.shape[2]
        q = jnp.einsum("bqm,mhd->bhqd", x, w_q)
        k = jnp.einsum("bkc,chd->bhkd", c_kv, w_uk)
        v = jnp.einsum("bkc,chd->bhkd", c_kv, w_uv)
        scores = jnp.einsum("bhqd,bhkd->bhqk", q, k) * (D ** -0.5)
        off = Sk - Sq
        qi = jnp.arange(Sq)[:, None]
        kj = jnp.arange(Sk)[None, :]
        cmask = kj <= (qi + off)
        scores = jnp.where(cmask[None, None], scores, -1e9)
        p = _softmax(scores, axis=-1)
        ctx = jnp.einsum("bhqk,bhkd->bhqd", p, v)
        return jnp.einsum("bhqd,hdm->bqm", ctx, w_o)

    def _B_ref(x, w1, b1, w2, b2):
        h = jnp.einsum("bsd,df->bsf", x, w1) + b1
        h = _gelu(h)
        return jnp.einsum("bsf,fd->bsd", h, w2) + b2

    x = A_x
    xn = _layernorm(x, axis=-1)
    s = _A_ref(xn, A_c_kv, A_w_q, A_w_uk, A_w_uv, A_w_o)
    g = _silu(_B_ref(xn, B_w1, B_b1, B_w2, B_b2))
    return x + s * g
```

```python
import jax
import jax.numpy as jnp
from jax import lax
import jax.experimental.pallas as pl
import jax.experimental.pallas.tpu as pltpu

_NT = (((1,), (1,)), ((), ()))
_F32 = jnp.float32
_BF16 = jnp.bfloat16

_WQ_CH = 512
_WUK_CH = 512
_WUV_CH = 512
_KV_DMA = 8192
_KV_CH = 2048
_WO_CHUNKS = ((0, 12), (12, 22), (22, 28), (28, 31), (31, 32))


def _gelu_tanh(x):
    return 0.5 * x * (1.0 + jnp.tanh(0.7978845608028654 * (x + 0.044715 * (x * x * x))))


def _make_kernel(B, H, Sk, D, M, Dc, F):
    HP = H // 2
    n_wq = M // _WQ_CH
    n_wuk = Dc // _WUK_CH
    n_wuv = Dc // _WUV_CH
    n_kv = Sk // _KV_CH
    n_kvd = Sk // _KV_DMA
    spd = _KV_DMA // _KV_CH
    scale = float(D) ** -0.5

    def kernel(x_hbm, ckv_hbm, wq_hbm, wuk_hbm, wuv_hbm, wo_hbm, w1_hbm, b1_hbm, w2_hbm, b2_hbm,
               o_hbm,
               x_v, b1_v, b2_v, wq_v, wuk_v, wuv_v, wo_v, w1_v, w2_v, ckv_v,
               ql_s, cl_s, l3_s, o_v,
               sem_small, sem_wq, sem_wuk, sem_kv, sem_wuv, sem_mlp, sem_wo, sem_out):

        cp_x = pltpu.make_async_copy(x_hbm, x_v, sem_small.at[0])
        cp_b1 = pltpu.make_async_copy(b1_hbm, b1_v, sem_small.at[1])
        cp_b2 = pltpu.make_async_copy(b2_hbm, b2_v, sem_small.at[2])

        def rows_cp(hbm, vm, sem, i, ch):
            return pltpu.make_async_copy(hbm.at[pl.ds(i * ch, ch)], vm.at[pl.ds(i * ch, ch)], sem.at[i])

        def kv_cp(b, j):
            return pltpu.make_async_copy(
                ckv_hbm.at[b, pl.ds(j * _KV_DMA, _KV_DMA)], ckv_v.at[b, pl.ds(j * _KV_DMA, _KV_DMA)],
                sem_kv.at[b * n_kvd + j])

        cp_w1 = pltpu.make_async_copy(w1_hbm, w1_v, sem_mlp.at[0])
        cp_w2 = pltpu.make_async_copy(w2_hbm, w2_v, sem_mlp.at[1])

        def wo_cp(i):
            lo, hi = _WO_CHUNKS[i]
            return pltpu.make_async_copy(wo_hbm.at[lo:hi], wo_v.at[lo:hi], sem_wo.at[i])

        order = [rows_cp(wq_hbm, wq_v, sem_wq, i, _WQ_CH) for i in range(n_wq)]
        order += [cp_x]
        order += [rows_cp(wuk_hbm, wuk_v, sem_wuk, i, _WUK_CH) for i in range(n_wuk)]
        order += [kv_cp(b, j) for b in range(B) for j in range(n_kvd)]
        order += [rows_cp(wuv_hbm, wuv_v, sem_wuv, i, _WUV_CH) for i in range(n_wuv)]
        order += [cp_b1, cp_w1, cp_b2, cp_w2]
        order += [wo_cp(i) for i in range(len(_WO_CHUNKS))]

        def issue(i, c):
            for k, cp in enumerate(order):
                pl.when(i == k)(cp.start)
            return c

        lax.fori_loop(0, len(order), issue, 0)

        cp_x.wait()
        xall = x_v[...].astype(_F32)
        xs = [xall[b:b + 1] for b in range(B)]
        xrows = []
        for b in range(B):
            xb = xs[b]
            mu = jnp.mean(xb, axis=-1, keepdims=True)
            xc = xb - mu
            var = jnp.mean(xc * xc, axis=-1, keepdims=True)
            xrows.append(xc * lax.rsqrt(var + 1e-5))
        row8 = lax.broadcasted_iota(jnp.int32, (8, M), 0)
        xn8 = jnp.zeros((8, M), _F32)
        for b in range(B):
            xn8 = jnp.where((row8 >> 1) == b, jnp.broadcast_to(xrows[b], (8, M)), xn8)
        xn8 = xn8.astype(_BF16)

        r_e = lax.broadcasted_iota(jnp.int32, (128, 256), 0)
        c_e = lax.broadcasted_iota(jnp.int32, (128, 256), 1)
        E0 = jnp.where((c_e >> 1) == r_e, 1.0, 0.0).astype(_BF16)
        r_s = lax.broadcasted_iota(jnp.int32, (256, 128), 0)
        c_s = lax.broadcasted_iota(jnp.int32, (256, 128), 1)
        S0 = jnp.where((r_s >> 1) == c_s, 1.0, 0.0).astype(_BF16)

        rr8 = lax.broadcasted_iota(jnp.int32, (8, 256), 0)
        cc8 = lax.broadcasted_iota(jnp.int32, (8, 256), 1)
        par_ok8 = (rr8 & 1) == (cc8 & 1)

        wq_u = wq_v.bitcast(jnp.uint32)
        q_acc = [jnp.zeros((8, D), _F32) for _ in range(HP)]
        for i in range(n_wq):
            rows_cp(wq_hbm, wq_v, sem_wq, i, _WQ_CH).wait()
            for sub in range(_WQ_CH // 128):
                m0 = i * _WQ_CH + sub * 128
                xe = jnp.dot(xn8[:, m0:m0 + 128], E0, preferred_element_type=_F32)
                l1 = jnp.where(par_ok8, xe, 0.0).astype(_BF16)
                for hp in range(HP):
                    wb = pltpu.bitcast(wq_u[m0:m0 + 128, hp, :], _BF16)
                    q_acc[hp] = q_acc[hp] + jnp.dot(l1, wb, preferred_element_type=_F32)
        q_bf = [a.astype(_BF16) for a in q_acc]

        wuk_u = wuk_v.bitcast(jnp.uint32)
        for i in range(n_wuk):
            rows_cp(wuk_hbm, wuk_v, sem_wuk, i, _WUK_CH).wait()
            for sub in range(_WUK_CH // 128):
                c0 = i * _WUK_CH + sub * 128
                outs = []
                for hp in range(HP):
                    wb = pltpu.bitcast(wuk_u[c0:c0 + 128, hp, :], _BF16)
                    o = lax.dot_general(q_bf[hp], wb, _NT, preferred_element_type=_F32)
                    outs.append(jnp.where(par_ok8, o * scale, 0.0))
                xj = jnp.concatenate(outs, axis=0).astype(_BF16)
                ql_s[c0 // 128] = jnp.dot(xj, S0, preferred_element_type=_F32)

        for b in range(B):
            ql = jnp.concatenate(
                [jnp.concatenate([ql_s[j, pl.ds(2 * b + p, HP, stride=8), :] for p in range(2)], axis=0)
                 for j in range(Dc // 128)], axis=1).astype(_BF16)

            def step(j, carry, b=b, ql=ql):
                m_i, l_i, acc = carry

                @pl.when(j % spd == 0)
                def _():
                    kv_cp(b, j // spd).wait()

                c = ckv_v[b, pl.ds(pl.multiple_of(j * _KV_CH, _KV_CH), _KV_CH), :]
                s = lax.dot_general(ql, c, _NT, preferred_element_type=_F32)
                m_new = jnp.maximum(m_i, jnp.max(s, axis=-1, keepdims=True))
                alpha = jnp.exp(m_i - m_new)
                p = jnp.exp(s - m_new)
                l_new = alpha * l_i + jnp.sum(p, axis=-1, keepdims=True)
                acc = alpha * acc + jnp.dot(p.astype(_BF16), c, preferred_element_type=_F32)
                return m_new, l_new, acc

            init = (jnp.full((H, 1), -1e30, _F32), jnp.zeros((H, 1), _F32), jnp.zeros((H, Dc), _F32))
            _, l_f, acc_f = lax.fori_loop(0, n_kv, step, init)
            cl_s[b * H:(b + 1) * H, :] = acc_f / l_f

        rr64 = lax.broadcasted_iota(jnp.int32, (B * H, 256), 0)
        cc64 = lax.broadcasted_iota(jnp.int32, (B * H, 256), 1)
        par_ok64 = ((rr64 // HP) & 1) == (cc64 & 1)
        for j in range(Dc // 128):
            cx = jnp.dot(cl_s[:, j * 128:(j + 1) * 128].astype(_BF16), E0, preferred_element_type=_F32)
            cx = jnp.where(par_ok64, cx, 0.0)
            l3_s[2 * j] = cx[:, :128]
            l3_s[2 * j + 1] = cx[:, 128:]

        wuv_u = wuv_v.bitcast(jnp.uint32)
        ctx_acc = [jnp.zeros((2 * B, D), _F32) for _ in range(HP)]
        for i in range(n_wuv):
            rows_cp(wuv_hbm, wuv_v, sem_wuv, i, _WUV_CH).wait()
            for sub in range(_WUV_CH // 128):
                c0 = i * _WUV_CH + sub * 128
                for hp in range(HP):
                    l3 = jnp.concatenate([l3_s[2 * (c0 // 128) + t, pl.ds(hp, 2 * B, stride=HP), :] for t in range(2)], axis=1).astype(_BF16)
                    wb = pltpu.bitcast(wuv_u[c0:c0 + 128, hp, :], _BF16)
                    ctx_acc[hp] = ctx_acc[hp] + jnp.dot(l3, wb, preferred_element_type=_F32)

        cp_b1.wait()
        cp_b2.wait()
        cp_w1.wait()
        b1 = b1_v[...].astype(_F32).reshape(1, F)
        hid = jnp.dot(xn8, w1_v[...], preferred_element_type=_F32) + b1
        hid = _gelu_tanh(hid).astype(_BF16)
        cp_w2.wait()
        b2 = b2_v[...].astype(_F32).reshape(1, M)
        gate = jnp.dot(hid, w2_v[...], preferred_element_type=_F32) + b2
        gate = gate * jax.nn.sigmoid(gate)

        rows4 = lax.broadcasted_iota(jnp.int32, (2 * B, D), 0)
        lo_parts = []
        for hp in range(HP):
            for p in range(2):
                lo_parts.append(jnp.where((rows4 & 1) == p, ctx_acc[hp], 0.0).astype(_BF16))
        out = jnp.zeros((2 * B, M), _F32)
        for i, (lo, hi) in enumerate(_WO_CHUNKS):
            wo_cp(i).wait()
            lhs = jnp.concatenate(lo_parts[lo:hi], axis=1)
            rhs = wo_v[lo:hi].reshape((hi - lo) * D, M)
            out = out + jnp.dot(lhs, rhs, preferred_element_type=_F32)

        for b in range(B):
            s_b = out[2 * b:2 * b + 1] + out[2 * b + 1:2 * b + 2]
            o_v[b:b + 1, :] = (xs[b] + s_b * gate[2 * b:2 * b + 1]).astype(o_v.dtype)
        cp_o = pltpu.make_async_copy(o_v, o_hbm, sem_out)
        cp_o.start()
        cp_o.wait()

    return kernel, (n_wq, n_wuk, n_kvd, n_wuv)


@jax.jit
def pallas_recurrent_scan__compressed_kv_cla__dense_activation_gelu__decode_kernel(
    A_x: jax.Array,
    A_c_kv: jax.Array,
    A_w_q: jax.Array,
    A_w_uk: jax.Array,
    A_w_uv: jax.Array,
    A_w_o: jax.Array,
    B_x: jax.Array,
    B_w1: jax.Array,
    B_b1: jax.Array,
    B_w2: jax.Array,
    B_b2: jax.Array,
):
    del B_x
    B, Sq, M = A_x.shape
    _, Sk, Dc = A_c_kv.shape
    _, H, D = A_w_q.shape
    F = B_w1.shape[1]
    kernel, (n_wq, n_wuk, n_kv, n_wuv) = _make_kernel(B, H, Sk, D, M, Dc, F)

    any_spec = pl.BlockSpec(memory_space=pl.ANY)
    out = pl.pallas_call(
        kernel,
        in_specs=[any_spec] * 10,
        out_specs=any_spec,
        out_shape=jax.ShapeDtypeStruct((B * Sq, M), A_x.dtype),
        scratch_shapes=[
            pltpu.VMEM((B * Sq, M), A_x.dtype),
            pltpu.VMEM(B_b1.shape, B_b1.dtype),
            pltpu.VMEM(B_b2.shape, B_b2.dtype),
            pltpu.VMEM(A_w_q.shape, A_w_q.dtype),
            pltpu.VMEM(A_w_uk.shape, A_w_uk.dtype),
            pltpu.VMEM(A_w_uv.shape, A_w_uv.dtype),
            pltpu.VMEM(A_w_o.shape, A_w_o.dtype),
            pltpu.VMEM(B_w1.shape, B_w1.dtype),
            pltpu.VMEM(B_w2.shape, B_w2.dtype),
            pltpu.VMEM(A_c_kv.shape, A_c_kv.dtype),
            pltpu.VMEM((Dc // 128, 8 * (H // 2), 128), _F32),
            pltpu.VMEM((B * H, Dc), _F32),
            pltpu.VMEM((2 * Dc // 128, B * H, 128), _F32),
            pltpu.VMEM((B * Sq, M), A_x.dtype),
            pltpu.SemaphoreType.DMA((3,)),
            pltpu.SemaphoreType.DMA((n_wq,)),
            pltpu.SemaphoreType.DMA((n_wuk,)),
            pltpu.SemaphoreType.DMA((B * n_kv,)),
            pltpu.SemaphoreType.DMA((n_wuv,)),
            pltpu.SemaphoreType.DMA((2,)),
            pltpu.SemaphoreType.DMA((len(_WO_CHUNKS),)),
            pltpu.SemaphoreType.DMA,
        ],
        compiler_params=pltpu.CompilerParams(vmem_limit_bytes=100 * 1024 * 1024),
    )(A_x.reshape(B * Sq, M), A_c_kv, A_w_q, A_w_uk, A_w_uv, A_w_o, B_w1, B_b1, B_w2, B_b2)
    return out.reshape(B, Sq, M)
```
